```python
import os as _os
_os.environ.setdefault("JAX_PLATFORMS", "cpu")
import jax
import jax.numpy as jnp

def _softmax(x, axis=-1):
    return jax.nn.softmax(x, axis=axis)
def _gelu(x):
    return jax.nn.gelu(x, approximate=True)
def _silu(x):
    return jax.nn.silu(x)
def _sigmoid(x):
    return jax.nn.sigmoid(x)
def _layernorm(x, axis=-1, eps=1e-5):
    m = jnp.mean(x, axis=axis, keepdims=True)
    v = jnp.var(x, axis=axis, keepdims=True)
    return (x - m) / jnp.sqrt(v + eps)
def _scatter_add(tgt, idx, src, axis=0):
    return tgt.at[idx].add(src)
def _segment_sum(src, seg, n):
    return jax.ops.segment_sum(src, seg, n)
class _Rng:
    def __init__(self, key):
        self._k = key
    def _next(self):
        self._k, sub = jax.random.split(self._k)
        return sub
    def normal(self, shape):
        return jax.random.normal(self._next(), shape, dtype=jnp.bfloat16)
    def randint(self, lo, hi, shape):
        return jax.random.randint(self._next(), shape, lo, hi, dtype=jnp.int32)
    def uniform(self, shape, lo=0.0, hi=1.0):
        return jax.random.uniform(self._next(), shape, jnp.bfloat16, lo, hi)
    def permutation(self, n):
        return jax.random.permutation(self._next(), n)


kernel_name = 'interleave_layers__sliding_local_dilated__softmax_full_mha__prompt'

def setup_inputs():
    _rng = _Rng(jax.random.key(int.from_bytes(__import__("os").urandom(4), "little")))
    _w = (lambda a: (lambda t: t.astype(jnp.bfloat16) if jnp.issubdtype(t.dtype, jnp.floating) else t)(jnp.asarray(a)))
    def _A_setup():
        B, S, D = 1, 2048, 512
        return {
            "x": _w((lambda *s: _rng.normal(s) * 0.05)(B, S, D)),
            "wqkv": _w((lambda *s: _rng.normal(s) * 0.05)(D, 3 * D)),
            "wo": _w((lambda *s: _rng.normal(s) * 0.05)(D, D)),
        }
    _A_in = _A_setup()

    def _B_setup():
        B, S, D = 1, 2048, 512
        return {
            "x": _w((lambda *s: _rng.normal(s) * 0.05)(B, S, D)),
            "wqkv": _w((lambda *s: _rng.normal(s) * 0.05)(D, 3 * D)),
            "wo": _w((lambda *s: _rng.normal(s) * 0.05)(D, D)),
        }
    _B_in = _B_setup()

    return {
        "A_x": _A_in["x"],
        "A_wqkv": _A_in["wqkv"],
        "A_wo": _A_in["wo"],
        "B_x": _B_in["x"],
        "B_wqkv": _B_in["wqkv"],
        "B_wo": _B_in["wo"],
    }

def reference(A_x, A_wqkv, A_wo, B_x, B_wqkv, B_wo):
    def _A_ref(x, wqkv, wo):
        B, S, D = x.shape
        H = 32; Dh = D // H
        W, dil = 8, 2
        qkv = (lambda x, *d: x.transpose(*d))((x @ wqkv).reshape(B, S, 3, H, Dh), 2, 0, 3, 1, 4)
        q, k, v = qkv[0], qkv[1], qkv[2]
        scale = Dh ** -0.5
        pos = jnp.arange(S)
        off = jnp.arange(W) * dil
        idx = pos[:, None] - off[None, :]
        mask = idx >= 0
        idx_c = jnp.where(mask, idx, 0).reshape(-1)
        kg = k[:, :, idx_c, :].reshape(B, H, S, W, Dh)
        vg = v[:, :, idx_c, :].reshape(B, H, S, W, Dh)
        logits = jnp.einsum("bhsd,bhswd->bhsw", q, kg) * scale
        logits = jnp.where(mask[None, None, :, :], logits, -1e9)
        attn = _softmax(logits, axis=-1)
        o = jnp.einsum("bhsw,bhswd->bhsd", attn, vg)
        return (lambda x, *d: x.transpose(*d))(o, 0, 2, 1, 3).reshape(B, S, D) @ wo

    def _B_ref(x, wqkv, wo):
        B, S, D = x.shape
        H = 32; Dh = D // H
        qkv = (lambda x, *d: x.transpose(*d))((x @ wqkv).reshape(B, S, 3, H, Dh), 2, 0, 3, 1, 4)
        q, k, v = qkv[0], qkv[1], qkv[2]
        scale = Dh ** -0.5
        scores = jnp.einsum("bhqd,bhkd->bhqk", q, k) * scale
        p = _softmax(scores, axis=-1)
        o = jnp.einsum("bhqk,bhkd->bhqd", p, v)
        return (lambda x, *d: x.transpose(*d))(o, 0, 2, 1, 3).reshape(B, S, D) @ wo

    x = A_x
    x = x + _A_ref(_layernorm(x, axis=-1), A_wqkv, A_wo)
    x = x + _B_ref(_layernorm(x, axis=-1), B_wqkv, B_wo)
    x = x + _A_ref(_layernorm(x, axis=-1), A_wqkv, A_wo)
    x = x + _B_ref(_layernorm(x, axis=-1), B_wqkv, B_wo)
    return x
```

```python
import jax
import jax.numpy as jnp
import jax.experimental.pallas as pl
import jax.experimental.pallas.tpu as pltpu

S, D, H, DH = 2048, 512, 32, 16
WIN = 8
NBLK = S // 128
LOG2E = 1.4426950408889634
QSCALE = DH ** -0.5 * LOG2E
MASKED = -1e9 * LOG2E
EPS = 1e-5
SAFE_LOG2 = 40.0

PIECE = 128
HEADS_PER_TRIP = 4
A_QKV, A_OUT, B_QKV, B_OUT, SPARE = 0, 3, 4, 7, 8

bf16, f32, u32 = jnp.bfloat16, jnp.float32, jnp.uint32
PITCH = 17


def _as_bf16(words):
    return pltpu.bitcast(words, bf16)


def _as_words(x):
    return pltpu.bitcast(x.astype(bf16), u32)


def _pack_pair(lo, hi):
    return pltpu.pack_elementwise([lo, hi], packed_dtype=bf16)


def _lanes(parts):
    return jnp.concatenate(parts, axis=1)


def _tile(x, t):
    return x[:, t * 128:(t + 1) * 128]


def _fold_rows(x):
    parts = [x[r:r + 8] for r in range(0, x.shape[0], 8)]
    while len(parts) > 1:
        parts = [a + b for a, b in zip(parts[0::2], parts[1::2])]
    return parts[0]


def _layernorm_tasks(x_refs, totals, out_refs, parts):
    mean, squares, scale = {}, {}, {}
    blocks = range(len(x_refs))

    def center(k):
        for t in blocks:
            if k == 0:
                mean[t] = jnp.broadcast_to(jnp.sum(totals(t), axis=0, keepdims=True) * (1.0 / D), (8, 128))
        for r in range(k * D // 8 // parts, (k + 1) * D // 8 // parts):
            for t in blocks:
                xc = x_refs[t][8 * r:8 * r + 8, :] - mean[t]
                squares[t] = xc * xc if r == 0 else squares[t] + xc * xc
        for t in blocks:
            if k == parts - 1:
                var = jnp.sum(squares[t], axis=0, keepdims=True) * (1.0 / D)
                scale[t] = jnp.broadcast_to(jax.lax.rsqrt(var + EPS), (8, 128))
        return pltpu.bitcast(squares[blocks[-1]], u32)

    def normalize(k):
        for r in range(k * D // 16 // parts, (k + 1) * D // 16 // parts):
            for t in blocks:
                even, odd = (x_refs[t][pl.ds(16 * r + i, 8, stride=2), :] for i in range(2))
                words = _pack_pair((even - mean[t]) * scale[t], (odd - mean[t]) * scale[t])
                out_refs[t][8 * r:8 * r + 8, :] = words
        return words

    return ([lambda y, k=k: center(k) for k in range(parts)]
            + [lambda y, k=k: normalize(k) for k in range(parts)])


def _kernel(x_hbm, wa_hbm, woa_hbm, wb_hbm, wob_hbm, out_hbm,
            io_buf, wa_in, wb_in, woa_in, wob_in, wtmp,
            w_all,
            x_t, xn, qa, kext, vext, oa,
            qf, qw, vw, kw, kvf, kvrot, ktmp, sqtmp, inv, norm2, ob, lb, krot, kb, qcur, krot2, kb2, qcur2,
            in_sem, out_sem):
    def lane_block_copies(src, dst, sem0):
        return [pltpu.make_async_copy(src.at[:, pl.ds(j * 128, 128)], dst.at[j], in_sem.at[sem0 + j])
                for j in range(4)]

    x_copies = lane_block_copies(x_hbm, io_buf, 0)
    wa_copies = [pltpu.make_async_copy(wa_hbm.at[:, pl.ds(part * D, D)], wa_in.at[part], in_sem.at[4 + part])
                 for part in range(3)]
    late_copies = lane_block_copies(woa_hbm, woa_in, 7) + [
        pltpu.make_async_copy(wb_hbm, wb_in, in_sem.at[11]),
        pltpu.make_async_copy(wob_hbm, wob_in, in_sem.at[12])]

    io_words = io_buf.bitcast(u32)
    for cp in x_copies:
        cp.start()
    for j in range(4):
        x_copies[j].wait()
        if j == 0:
            for cp in wa_copies:
                cp.start()
        for i in range(8):
            w = io_words[j, pl.ds(i, 128, stride=8), :].T
            for par, bits in enumerate((w << 16, w & jnp.uint32(0xFFFF0000))):
                x_t[2 * par + i // 4][i % 4, j * 128:(j + 1) * 128, :] = pltpu.bitcast(bits, f32)
    for cp in late_copies:
        cp.start()
    for c in range(4):
        for task in _layernorm_tasks([x_t[c].at[t] for t in range(4)], lambda t, c=c: _fold_rows(x_t[c][t]),
                                     [xn[c].at[t] for t in range(4)], 1):
            task(None)

    for part in range(3):
        wa_copies[part].wait()
        for j in range(4):
            wt = wa_in[part, :, j * 128:(j + 1) * 128].astype(f32).T
            for kt in range(4):
                for hh in range(8):
                    wtmp[kt, pl.ds((8 * j + hh) * PITCH, DH), :] = _tile(wt, kt)[DH * hh:DH * (hh + 1)]
        for kt in range(4):
            rows = [wtmp[kt, pl.ds(d, H, stride=PITCH), :] for d in range(DH)]
            w_all[A_QKV + part, :, kt * 128:(kt + 1) * 128] = _as_words(jnp.concatenate(rows, axis=0))
    for cp in late_copies:
        cp.wait()

    def transpose_late_weights():
        woa_words = woa_in.bitcast(u32)
        for j in range(4):
            rows = [woa_words[j, pl.ds(dp, H, stride=8), :] for dp in range(8)]
            w_all[A_OUT, j * 64:(j + 1) * 64, :] = pltpu.bitcast(_as_bf16(jnp.concatenate(rows, axis=0)).T, u32)
        for part in range(3):
            for j in range(4):
                col = part * D + j * 128
                w_all[B_QKV + part, j * 64:(j + 1) * 64, :] = pltpu.bitcast(wb_in[:, col:col + 128].T, u32)
        for j in range(4):
            w_all[B_OUT, j * 64:(j + 1) * 64, :] = pltpu.bitcast(wob_in[:, j * 128:(j + 1) * 128].T, u32)

    lane = jax.lax.broadcasted_iota(jnp.int32, (8, 128), 1)

    piece_rows = range(0, D, PIECE)

    def project(slot, act, c, row):
        rhs = _as_bf16(_lanes([act[c][t] for t in range(4)]))
        return jnp.dot(_as_bf16(w_all[slot, row // 2:(row + PIECE) // 2, :]), rhs, preferred_element_type=f32)

    def local_qkv(c, part, row):
        par, i0, rows = c // 2, 4 * (c % 2), pl.ds(row, PIECE)
        y = project(A_QKV + part, xn, c, row)
        for t in range(4):
            i, yt = i0 + t, _tile(y, t)
            if part == 0:
                qa[par][1 + i, rows, :] = yt * QSCALE
                continue
            ext = kext if part == 1 else vext
            ext[par][7 + i, rows, :] = yt
            if i > 0:
                shifted = pltpu.roll(yt, 1, axis=1)
                if part == 2:
                    first = jax.lax.broadcasted_iota(jnp.int32, yt.shape, 1) == 0
                    shifted = jnp.where(first, vext[0][7, rows, :], shifted)
                ext[par][i - 1, rows, :] = shifted
        return y

    def local_attention(par, i, g):
        rows = [pl.ds(d * H + 8 * g, 8) for d in range(DH)]
        q = [qa[par][1 + i, r, :] for r in rows]
        logits = []
        for w in range(WIN):
            acc = q[0] * kext[par][7 + i - w, rows[0], :]
            for d in range(1, DH):
                acc = acc + q[d] * kext[par][7 + i - w, rows[d], :]
            logits.append(jnp.where(lane == 0, MASKED, acc) if w > i else acc)
        m = logits[0]
        for w in range(1, WIN):
            m = jnp.maximum(m, logits[w])
        p = [jnp.exp2(l - m) for l in logits]
        total = p[0]
        for w in range(1, WIN):
            total = total + p[w]
        inv = 1.0 / total
        p = [pw * inv for pw in p]
        for dp in range(DH // 2):
            pair = []
            for d in (2 * dp, 2 * dp + 1):
                acc = p[0] * vext[par][7 + i, rows[d], :]
                for w in range(1, WIN):
                    acc = acc + p[w] * vext[par][7 + i - w, rows[d], :]
                pair.append(acc)
            words = _pack_pair(*pair)
            oa[2 * par + i // 4][i % 4, pl.ds(dp * H + 8 * g, 8), :] = words
        return words

    totals = {}

    def out_proj(slot, c, row):
        rows = pl.ds(row, PIECE)
        y = project(slot, oa, c, row)
        for t in range(4):
            xb = x_t[c][t, rows, :] + _tile(y, t)
            x_t[c][t, rows, :] = xb
            totals[c, t] = _fold_rows(xb) if row == 0 else totals[c, t] + _fold_rows(xb)
        return y

    def gated(ref, slot, task):
        def gated_task(y):
            if y is not None:
                ref[slot, 0:8, :] = y[-8:, 384:512]
            return task(y)
        return gated_task

    def norm_tasks(c, zero):
        tasks = _layernorm_tasks([x_t[c].at[t] for t in range(4)], lambda t: totals.pop((c, t)),
                                 [xn[c].at[t] for t in range(4)], 2)
        return [gated(x_t[c], 4 - zero, task) for task in tasks]

    def out_products(slot, c):
        return [lambda row=row: out_proj(slot, c, row) for row in piece_rows]

    def run(products, tasks=()):
        done = 0
        for n, product in enumerate(products):
            y = product()
            while done < len(tasks) and done * len(products) < (n + 1) * len(tasks):
                tasks[done](y)
                done += 1

    def head_sums(ref, n):
        total = ref[pl.ds(0, n, stride=8), :]
        for r in range(1, 8):
            total = total + ref[pl.ds(r, n, stride=8), :]
        return total

    def full_qkv(c, part, row):
        nh = PIECE // DH
        hs = pl.ds(row // DH, nh)
        y = project(B_QKV + part, xn, c, row)
        if part == 0:
            y = y * QSCALE
        for t in range(4):
            b, yt = 4 * c + t, _tile(y, t)
            if part < 2:
                sq = (yt * yt).reshape(nh, 2, 8, 128)
                sqtmp[t][0:8 * nh, :] = (sq[:, 0] + sq[:, 1]).reshape(8 * nh, 128)
                n2 = head_sums(sqtmp[t], nh)
                norm2[part, hs, :] = n2 if b == 0 else jnp.maximum(norm2[part, hs, :], n2)
            if part == 0:
                qf[b, hs] = yt.reshape(nh, DH, 128)
                qw[b, hs] = _as_words(yt).reshape(nh, 8, 128)
            elif part == 2:
                vw[b, hs] = _as_words(yt).reshape(nh, 8, 128)
            else:
                g = row // 128
                ktmp[t][g] = yt.T
                even = ktmp[t][g, pl.ds(0, 64, stride=2), :]
                odd = ktmp[t][g, pl.ds(1, 64, stride=2), :]
                rows = []
                for r in range(8):
                    rows += [even[8 * r:8 * r + 8], odd[8 * r:8 * r + 8]]
                kw[g, b] = _as_words(jnp.concatenate(rows, axis=0))
                kvf[g, b] = jnp.concatenate([even[0:8], odd[0:8]], axis=0)
        return y

    def head_shift(h):
        return (128 - DH * (h % 8)) % 128

    def q_operand(h, c):
        q = _lanes([qw[4 * c + t, h] for t in range(4)])
        return _as_bf16(jnp.concatenate([q, jnp.zeros((56, 512), u32)], axis=0))

    def stage_keys(h, j, dst):
        g, shift = h // 8, head_shift(h)
        dst[j, 8:64, :] = pltpu.roll(kw[g, j, 8:64, :], shift, axis=1)
        kvrot[j] = pltpu.roll(kvf[g, j], shift, axis=1)

    def splat_keys(d, blocks, dst):
        keys = jnp.concatenate([kvrot[j] for j in blocks], axis=0)
        splat = jnp.broadcast_to(keys[:, d:d + 1], keys.shape)
        for n, j in enumerate(blocks):
            dst[j, d] = splat[16 * n:16 * n + 16]

    def stage_queries(h, c, dst):
        for b in range(4 * c, 4 * c + 4):
            dst[:, b * 128:(b + 1) * 128] = qf[b, h]

    def fast_heads(heads):
        steps = [(u, c, j) for u in range(len(heads)) for c in range(4) for j in range(NBLK)]
        scores, probs, sums = {}, {}, {}
        terms = [(n, t, d) for n in range(len(steps)) for t in range(4) for d in range(DH)]
        partial, state = {}, dict(terms=0, pairs=0)

        def emit(n, row, t, s0, s1):
            u, c, j = steps[n]
            p0, p1 = jnp.exp2(s0), jnp.exp2(s1)
            sums[u, c, t] = p0 + p1 if (u, c, t) not in sums else (sums[u, c, t] + p0) + p1
            probs[n, row, t] = _pack_pair(p0, p1)

        def vector_term():
            n, t, d = terms[state["terms"]]
            u, c, j = steps[n]
            _, keys, queries = heads[u][1]
            col = (4 * c + t) * 128
            q = jnp.broadcast_to(queries[d:d + 1, col:col + 128], (8, 128))
            for odd in range(2):
                term = keys[j, d, 8 * odd:8 * odd + 8, :] * q
                partial[odd] = term if d == 0 else partial[odd] + term
            if d == DH - 1:
                emit(n, 0, t, partial[0], partial[1])
            state["terms"] += 1

        def exponentials(n):
            u, c, j = steps[n]
            h, _, h_next, nxt = heads[u]
            s = scores.pop(n)
            for r in range(7):
                for t in range(4):
                    while state["terms"] < len(terms) and state["terms"] * 28 <= state["pairs"] * 4 * DH:
                        vector_term()
                    emit(n, r + 1, t, _tile(s[16 * r:16 * r + 8], t), _tile(s[16 * r + 8:16 * r + 16], t))
                    state["pairs"] += 1
            while state["terms"] < len(terms) and terms[state["terms"]][0] <= n:
                vector_term()
            if j == NBLK - 1:
                for t in range(4):
                    lb[4 * c + t, pl.ds(pl.multiple_of(8 * h, 8), 8), :] = sums.pop((u, c, t))
            blocks = range(4 * c, 4 * c + 4)
            if j == 0:
                for block in blocks:
                    stage_keys(h_next, block, nxt[0])
            splat_keys(j, blocks, nxt[1])
            if j == 3:
                stage_queries(h_next, c, nxt[2])

        def weighted_values(n):
            u, c, j = steps[n]
            h = heads[u][0]
            p = jnp.concatenate([_lanes([probs.pop((n, r, t)) for t in range(4)]) for r in range(8)], axis=0)
            o = jnp.dot(_as_bf16(vw[j, h]), _as_bf16(p), preferred_element_type=f32)
            for t in range(4):
                ob[4 * c + t, h] = _tile(o, t) if j == 0 else ob[4 * c + t, h] + _tile(o, t)

        for n in range(len(steps) + 2):
            if n < len(steps):
                u, c, j = steps[n]
                h, (keys, _, _) = heads[u][:2]
                scores[n] = jnp.dot(_as_bf16(keys[j, 8:64, :]), q_operand(h, c), preferred_element_type=f32)
            if 0 <= n - 1 < len(steps):
                exponentials(n - 1)
            if n - 2 >= 0:
                weighted_values(n - 2)

    def fast_trip(i, carry):
        stages = ((krot, kb, qcur), (krot2, kb2, qcur2))
        first = HEADS_PER_TRIP * i
        fast_heads([(first + u, stages[u % 2], jnp.minimum(first + u + 1, H - 1), stages[1 - u % 2])
                    for u in range(HEADS_PER_TRIP)])
        return carry

    def guarded_head(h, carry):
        g, shift = h // 8, head_shift(h)

        def rotate(j, carry):
            krot[j] = pltpu.roll(kw[g, j], shift, axis=1)
            return carry

        jax.lax.fori_loop(0, NBLK, rotate, 0)

        def chunk(c, carry):
            q = q_operand(h, c)

            def block_scores(j):
                return jnp.dot(_as_bf16(krot[j]), q, preferred_element_type=f32)

            def running_max(j, m):
                return jnp.maximum(m, jnp.max(block_scores(j), axis=0, keepdims=True))

            m = jax.lax.fori_loop(0, NBLK, running_max, jnp.full((1, 512), -jnp.inf, f32))

            def accumulate(j, state):
                acc, total = state
                p = jnp.exp2(block_scores(j) - m)
                words = [_pack_pair(p[16 * r:16 * r + 8], p[16 * r + 8:16 * r + 16]) for r in range(8)]
                o = jnp.dot(_as_bf16(vw[j, h]), _as_bf16(jnp.concatenate(words, axis=0)),
                            preferred_element_type=f32)
                return acc + o, total + jnp.sum(p.reshape(16, 8, 512), axis=0)

            acc, total = jax.lax.fori_loop(
                0, NBLK, accumulate, (jnp.zeros((DH, 512), f32), jnp.zeros((8, 512), f32)))
            for t in range(4):
                ob[4 * c + t, h] = _tile(acc, t)
                lb[4 * c + t, pl.ds(pl.multiple_of(8 * h, 8), 8), :] = _tile(total, t)
            return carry

        return jax.lax.fori_loop(0, 4, chunk, carry)

    def full_attention():
        for j in range(NBLK):
            stage_keys(0, j, krot)
        for d in range(DH):
            splat_keys(d, range(NBLK), kb)
        for c in range(4):
            stage_queries(0, c, qcur)
        bound2 = jnp.max(norm2[0], axis=-1, keepdims=True) * jnp.max(norm2[1], axis=-1, keepdims=True)
        unsafe = jnp.max(jnp.where(bound2 <= SAFE_LOG2 * SAFE_LOG2, 0.0, 1.0))

        @pl.when(unsafe == 0.0)
        def _():
            jax.lax.fori_loop(0, H // HEADS_PER_TRIP, fast_trip, 0)

        @pl.when(unsafe != 0.0)
        def _():
            jax.lax.fori_loop(0, H, guarded_head, 0)

    def normalize_tasks(c):
        def task(y, t):
            b = 4 * c + t
            inv[c][t] = 1.0 / head_sums(lb.at[b], H)
            for h in range(H):
                scale = jnp.broadcast_to(inv[c][t, h:h + 1, :], (8, 128))
                even, odd = (ob[b, h, pl.ds(k, 8, stride=2), :] for k in range(2))
                words = _pack_pair(even * scale, odd * scale)
                oa[c][t, 8 * h:8 * h + 8, :] = words
            return words
        return [lambda y, t=t: task(y, t) for t in range(4)]

    def full_out(zero):
        for task in normalize_tasks(0):
            task(None)
        run(out_products(B_OUT, 0), normalize_tasks(1))
        run(out_products(B_OUT, 1), norm_tasks(0, zero) + normalize_tasks(2))
        run(out_products(B_OUT, 2), norm_tasks(1, zero) + normalize_tasks(3))
        run(out_products(B_OUT, 3), norm_tasks(2, zero))
        for task in norm_tasks(3, zero):
            task(None)

    def write_output():
        for c in (0, 2, 1, 3):
            for task in normalize_tasks(c):
                task(None)
        copies = []
        for j in range(4):
            for c in range(2):
                even, odd = project(B_OUT, oa, c, j * 128), project(B_OUT, oa, c + 2, j * 128)
                rows = pl.ds(j * 128, 128)
                for t in range(4):
                    words = _pack_pair(x_t[c][t, rows, :] + _tile(even, t), x_t[2 + c][t, rows, :] + _tile(odd, t))
                    io_words[j, pl.ds(4 * c + t, 128, stride=8), :] = words.T
            cp = pltpu.make_async_copy(io_buf.at[j], out_hbm.at[:, pl.ds(j * 128, 128)], out_sem.at[j])
            cp.start()
            copies.append(cp)
        for cp in copies:
            cp.wait()

    def dense_part(zero):
        def products(fn, c):
            return [lambda part=part, row=row: fn(c, part, row) for part in range(3) for row in piece_rows]

        def attention_task(par, i, g):
            return gated(qa[par], zero, lambda y: local_attention(par, i, g))

        def with_norm(c):
            outs = out_products(A_OUT, c)

            def last(product=outs[-1]):
                y = product()
                for task in norm_tasks(c, zero):
                    task(None)
                return y
            return outs[:-1] + [last]

        tasks = [[attention_task(par, i, g) for i in range(8) for g in range(4)] for par in range(2)]
        transpose_late_weights()
        run(products(local_qkv, 0) + products(local_qkv, 1))
        queue = products(local_qkv, 2) + products(local_qkv, 3)
        run(queue[:-2], tasks[0])
        run(queue[-2:])
        queue = with_norm(0) + with_norm(1) + products(full_qkv, 0) + products(full_qkv, 1)
        run(queue[:4])
        run(queue[4:-2], tasks[1])
        run(queue[-2:] + with_norm(2) + with_norm(3) + products(full_qkv, 2) + products(full_qkv, 3))

    def layer_pair(rep, carry):
        zero = rep // 2
        dense_part(zero)
        full_attention()

        @pl.when(rep == 0)
        def _():
            full_out(zero)

        return carry

    jax.lax.fori_loop(0, 2, layer_pair, 0)
    write_output()


@jax.jit
def pallas_interleave_layers__sliding_local_dilated__softmax_full_mha__prompt_kernel(
    A_x: jax.Array,
    A_wqkv: jax.Array,
    A_wo: jax.Array,
    B_x: jax.Array,
    B_wqkv: jax.Array,
    B_wo: jax.Array,
):
    del B_x
    vmem = pltpu.VMEM
    scratch = [
        vmem((4, S, 128), bf16),
        vmem((3, D, D), bf16),
        vmem((D, 3 * D), bf16),
        vmem((4, D, 128), bf16),
        vmem((D, D), bf16),
        vmem((4, H * PITCH, 128), f32),
        vmem((9, D // 2, D), u32),
        [vmem((5, D, 128), f32)] * 4,
        [vmem((4, D // 2, 128), u32)] * 4,
        [vmem((9, D, 128), f32)] * 2,
        [vmem((15, D, 128), f32)] * 2,
        [vmem((15, D, 128), f32)] * 2,
        [vmem((4, D // 2, 128), u32)] * 4,
        vmem((NBLK, H, DH, 128), f32),
        vmem((NBLK, H, 8, 128), u32),
        vmem((NBLK, H, 8, 128), u32),
        vmem((4, NBLK, 64, 128), u32),
        vmem((4, NBLK, 16, 128), f32),
        vmem((NBLK, 16, 128), f32),
        [vmem((4, 128, 128), f32)] * 4,
        [vmem((8 * H, 128), f32)] * 4,
        [vmem((4, H, 128), f32)] * 4,
        vmem((2, H, 128), f32),
        vmem((NBLK, H, DH, 128), f32),
        vmem((NBLK, 8 * H, 128), f32),
        vmem((NBLK, 64, 128), u32),
        vmem((NBLK, DH, 16, 128), f32),
        vmem((DH, S), f32),
        vmem((NBLK, 64, 128), u32),
        vmem((NBLK, DH, 16, 128), f32),
        vmem((DH, S), f32),
        pltpu.SemaphoreType.DMA((13,)),
        pltpu.SemaphoreType.DMA((4,)),
    ]
    out = pl.pallas_call(
        _kernel,
        out_shape=jax.ShapeDtypeStruct((S, D), bf16),
        in_specs=[pl.BlockSpec(memory_space=pl.ANY)] * 5,
        out_specs=pl.BlockSpec(memory_space=pl.ANY),
        scratch_shapes=scratch,
        compiler_params=pltpu.CompilerParams(
            vmem_limit_bytes=100 * 1024 * 1024,
            flags={"XLA_TPU_EVENLY_DISTRIBUTE_CRITICAL_NODES": True},
        ),
    )(A_x.reshape(S, D), A_wqkv, A_wo, B_wqkv, B_wo)
    return out.reshape(A_x.shape)
```

```python
import jax
import jax.numpy as jnp
import jax.experimental.pallas as pl
import jax.experimental.pallas.tpu as pltpu

S, D, H, DH = 2048, 512, 32, 16
WIN = 8
NBLK = S // 128
LOG2E = 1.4426950408889634
QSCALE = DH ** -0.5 * LOG2E
MASKED = -1e9 * LOG2E
EPS = 1e-5
SAFE_LOG2 = 40.0

HEADS_PER_TRIP = 4
A_QKV, A_OUT, B_QKV, B_OUT = 0, 3, 4, 7

bf16, f32, u32 = jnp.bfloat16, jnp.float32, jnp.uint32
PITCH = 17


def _as_bf16(words):
    return pltpu.bitcast(words, bf16)


def _as_words(x):
    return pltpu.bitcast(x.astype(bf16), u32)


def _pack_pair(lo, hi):
    return pltpu.pack_elementwise([lo, hi], packed_dtype=bf16)


def _lanes(parts):
    return jnp.concatenate(parts, axis=1)


def _tile(x, t):
    return x[:, t * 128:(t + 1) * 128]


def _fold_rows(x):
    parts = [x[r:r + 8] for r in range(0, x.shape[0], 8)]
    while len(parts) > 1:
        parts = [a + b for a, b in zip(parts[0::2], parts[1::2])]
    return parts[0]


def _layernorm_tasks(x_refs, totals, out_refs, parts):
    mean, squares, scale = {}, {}, {}
    blocks = range(len(x_refs))

    def center(k):
        for t in blocks:
            if k == 0:
                mean[t] = jnp.broadcast_to(jnp.sum(totals(t), axis=0, keepdims=True) * (1.0 / D), (8, 128))
        for r in range(k * D // 8 // parts, (k + 1) * D // 8 // parts):
            for t in blocks:
                xc = x_refs[t][8 * r:8 * r + 8, :] - mean[t]
                squares[t] = xc * xc if r == 0 else squares[t] + xc * xc
        for t in blocks:
            if k == parts - 1:
                var = jnp.sum(squares[t], axis=0, keepdims=True) * (1.0 / D)
                scale[t] = jnp.broadcast_to(jax.lax.rsqrt(var + EPS), (8, 128))
        return pltpu.bitcast(squares[blocks[-1]], u32)

    def normalize(k):
        for r in range(k * D // 16 // parts, (k + 1) * D // 16 // parts):
            for t in blocks:
                even, odd = (x_refs[t][pl.ds(16 * r + i, 8, stride=2), :] for i in range(2))
                words = _pack_pair((even - mean[t]) * scale[t], (odd - mean[t]) * scale[t])
                out_refs[t][8 * r:8 * r + 8, :] = words
        return words

    return ([lambda y, k=k: center(k) for k in range(parts)]
            + [lambda y, k=k: normalize(k) for k in range(parts)])


def _kernel(x_hbm, wa_hbm, woa_hbm, wb_hbm, wob_hbm, out_hbm,
            io_buf, wa_in, wb_in, woa_in, wob_in, wtmp,
            w_all,
            x_t, xn, qa, kext, vext, oa,
            qf, qw, vw, kw, kvf, kvrot, ktmp, sqtmp, inv, norm2, ob, lb, krot, kb, qcur, krot2, kb2, qcur2,
            in_sem, out_sem):
    def lane_block_copies(src, dst, sem0):
        return [pltpu.make_async_copy(src.at[:, pl.ds(j * 128, 128)], dst.at[j], in_sem.at[sem0 + j])
                for j in range(4)]

    x_copies = lane_block_copies(x_hbm, io_buf, 0)
    wa_copies = [pltpu.make_async_copy(wa_hbm.at[:, pl.ds(part * D, D)], wa_in.at[part], in_sem.at[4 + part])
                 for part in range(3)]
    late_copies = lane_block_copies(woa_hbm, woa_in, 7) + [
        pltpu.make_async_copy(wb_hbm, wb_in, in_sem.at[11]),
        pltpu.make_async_copy(wob_hbm, wob_in, in_sem.at[12])]

    io_words = io_buf.bitcast(u32)
    for cp in x_copies:
        cp.start()
    for j in range(4):
        x_copies[j].wait()
        if j == 0:
            for cp in wa_copies:
                cp.start()
        for i in range(8):
            w = io_words[j, pl.ds(i, 128, stride=8), :].T
            for par, bits in enumerate((w << 16, w & jnp.uint32(0xFFFF0000))):
                x_t[2 * par + i // 4][i % 4, j * 128:(j + 1) * 128, :] = pltpu.bitcast(bits, f32)
    for cp in late_copies:
        cp.start()
    for c in range(4):
        for task in _layernorm_tasks([x_t[c].at[t] for t in range(4)], lambda t, c=c: _fold_rows(x_t[c][t]),
                                     [xn[c].at[t] for t in range(4)], 1):
            task(None)

    for part in range(3):
        wa_copies[part].wait()
        for j in range(4):
            wt = wa_in[part, :, j * 128:(j + 1) * 128].astype(f32).T
            for kt in range(4):
                for hh in range(8):
                    wtmp[kt, pl.ds((8 * j + hh) * PITCH, DH), :] = _tile(wt, kt)[DH * hh:DH * (hh + 1)]
        for kt in range(4):
            rows = [wtmp[kt, pl.ds(d, H, stride=PITCH), :] for d in range(DH)]
            w_all[A_QKV + part, :, kt * 128:(kt + 1) * 128] = _as_words(jnp.concatenate(rows, axis=0))
    def transpose_late_weights():
        for cp in late_copies:
            cp.wait()
        woa_words = woa_in.bitcast(u32)
        for j in range(4):
            rows = [woa_words[j, pl.ds(dp, H, stride=8), :] for dp in range(8)]
            w_all[A_OUT, j * 64:(j + 1) * 64, :] = pltpu.bitcast(_as_bf16(jnp.concatenate(rows, axis=0)).T, u32)
        for part in range(3):
            for j in range(4):
                col = part * D + j * 128
                w_all[B_QKV + part, j * 64:(j + 1) * 64, :] = pltpu.bitcast(wb_in[:, col:col + 128].T, u32)
        for j in range(4):
            w_all[B_OUT, j * 64:(j + 1) * 64, :] = pltpu.bitcast(wob_in[:, j * 128:(j + 1) * 128].T, u32)

    lane = jax.lax.broadcasted_iota(jnp.int32, (8, 128), 1)

    def project(slot, act, c, row, size):
        rhs = _as_bf16(_lanes([act[c][t] for t in range(4)]))
        return jnp.dot(_as_bf16(w_all[slot, row // 2:(row + size) // 2, :]), rhs, preferred_element_type=f32)

    def local_qkv(c, part, row, size):
        par, i0, rows = c // 2, 4 * (c % 2), pl.ds(row, size)
        y = project(A_QKV + part, xn, c, row, size)
        for t in range(4):
            i, yt = i0 + t, _tile(y, t)
            if part == 0:
                qa[par][1 + i, rows, :] = yt * QSCALE
                continue
            ext = kext if part == 1 else vext
            ext[par][7 + i, rows, :] = yt
            if i > 0:
                shifted = pltpu.roll(yt, 1, axis=1)
                if part == 2:
                    first = jax.lax.broadcasted_iota(jnp.int32, yt.shape, 1) == 0
                    shifted = jnp.where(first, vext[0][7, rows, :], shifted)
                ext[par][i - 1, rows, :] = shifted
        return y

    def local_attention(par, i, g):
        rows = [pl.ds(d * H + 8 * g, 8) for d in range(DH)]
        q = [qa[par][1 + i, r, :] for r in rows]
        logits = []
        for w in range(WIN):
            acc = q[0] * kext[par][7 + i - w, rows[0], :]
            for d in range(1, DH):
                acc = acc + q[d] * kext[par][7 + i - w, rows[d], :]
            logits.append(jnp.where(lane == 0, MASKED, acc) if w > i else acc)
        m = logits[0]
        for w in range(1, WIN):
            m = jnp.maximum(m, logits[w])
        p = [jnp.exp2(l - m) for l in logits]
        total = p[0]
        for w in range(1, WIN):
            total = total + p[w]
        inv = 1.0 / total
        p = [pw * inv for pw in p]
        for dp in range(DH // 2):
            pair = []
            for d in (2 * dp, 2 * dp + 1):
                acc = p[0] * vext[par][7 + i, rows[d], :]
                for w in range(1, WIN):
                    acc = acc + p[w] * vext[par][7 + i - w, rows[d], :]
                pair.append(acc)
            words = _pack_pair(*pair)
            oa[2 * par + i // 4][i % 4, pl.ds(dp * H + 8 * g, 8), :] = words
        return words

    moments, pivots = {}, {}

    def out_proj(slot, c, row, size):
        rows = pl.ds(row, size)
        y = project(slot, oa, c, row, size)
        for t in range(4):
            xb = x_t[c][t, rows, :] + _tile(y, t)
            x_t[c][t, rows, :] = xb
            if row == 0:
                pivots[c, t] = jnp.broadcast_to(xb[0:1], (8, 128))
            xc = xb - jnp.concatenate([pivots[c, t]] * (size // 8), axis=0)
            first, second = _fold_rows(xc), _fold_rows(xc * xc)
            moments[c, t] = (first, second) if row == 0 else (moments[c, t][0] + first, moments[c, t][1] + second)
        return y

    def gated(ref, slot, task):
        def gated_task(y):
            if y is not None:
                ref[slot, 0:8, :] = y[-8:, 384:512]
            return task(y)
        return gated_task

    def norm_tasks(c, zero):
        stats = {}

        def normalize(k):
            for t in range(4):
                if k == 0:
                    shift, square = (jnp.sum(v, axis=0, keepdims=True) * (1.0 / D) for v in moments.pop((c, t)))
                    var = jnp.maximum(square - shift * shift, 0.0)
                    stats[t] = (pivots.pop((c, t)) + shift, jnp.broadcast_to(jax.lax.rsqrt(var + EPS), (8, 128)))
            for r in range(16 * k, 16 * k + 16):
                for t in range(4):
                    even, odd = (x_t[c][t, pl.ds(16 * r + i, 8, stride=2), :] for i in range(2))
                    mean, scale = stats[t]
                    xn[c][t, 8 * r:8 * r + 8, :] = _pack_pair((even - mean) * scale, (odd - mean) * scale)

        return [gated(x_t[c], 4 - zero, lambda y, k=k: normalize(k)) for k in range(2)]

    def out_products(slot, c):
        return [lambda row=row: out_proj(slot, c, row, 128) for row in range(0, D, 128)]

    def run(products, tasks=()):
        done = 0
        for n, product in enumerate(products):
            y = product()
            while done < len(tasks) and done * len(products) < (n + 1) * len(tasks):
                tasks[done](y)
                done += 1

    def head_sums(ref, n):
        total = ref[pl.ds(0, n, stride=8), :]
        for r in range(1, 8):
            total = total + ref[pl.ds(r, n, stride=8), :]
        return total

    def full_qkv(c, part, row, size):
        nh = size // DH
        hs = pl.ds(row // DH, nh)
        y = project(B_QKV + part, xn, c, row, size)
        if part == 0:
            y = y * QSCALE
        for t in range(4):
            b, yt = 4 * c + t, _tile(y, t)
            if part < 2:
                sq = (yt * yt).reshape(nh, 2, 8, 128)
                sqtmp[t][0:8 * nh, :] = (sq[:, 0] + sq[:, 1]).reshape(8 * nh, 128)
                n2 = head_sums(sqtmp[t], nh)
                norm2[part, hs, :] = n2 if b == 0 else jnp.maximum(norm2[part, hs, :], n2)
            if part == 0:
                qf[b, hs] = yt.reshape(nh, DH, 128)
                qw[b, hs] = _as_words(yt).reshape(nh, 8, 128)
            elif part == 2:
                vw[b, hs] = _as_words(yt).reshape(nh, 8, 128)
            else:
                for k in range(size // 128):
                    g = row // 128 + k
                    ktmp[t][g] = yt[k * 128:(k + 1) * 128, :].T
                    even = ktmp[t][g, pl.ds(0, 64, stride=2), :]
                    odd = ktmp[t][g, pl.ds(1, 64, stride=2), :]
                    rows = []
                    for r in range(8):
                        rows += [even[8 * r:8 * r + 8], odd[8 * r:8 * r + 8]]
                    kw[g, b] = _as_words(jnp.concatenate(rows, axis=0))
                    kvf[g, b] = jnp.concatenate([even[0:8], odd[0:8]], axis=0)
        return y

    def head_shift(h):
        return (128 - DH * (h % 8)) % 128

    def q_operand(h, c):
        q = _lanes([qw[4 * c + t, h] for t in range(4)])
        return _as_bf16(jnp.concatenate([q, jnp.zeros((56, 512), u32)], axis=0))

    def stage_keys(h, j, dst):
        g, shift = h // 8, head_shift(h)
        dst[j, 8:64, :] = pltpu.roll(kw[g, j, 8:64, :], shift, axis=1)
        kvrot[j] = pltpu.roll(kvf[g, j], shift, axis=1)

    def splat_keys(d, blocks, dst):
        keys = jnp.concatenate([kvrot[j] for j in blocks], axis=0)
        splat = jnp.broadcast_to(keys[:, d:d + 1], keys.shape)
        for n, j in enumerate(blocks):
            dst[j, d] = splat[16 * n:16 * n + 16]

    def stage_queries(h, c, dst):
        for b in range(4 * c, 4 * c + 4):
            dst[:, b * 128:(b + 1) * 128] = qf[b, h]

    def fast_heads(heads):
        steps = [(u, c, j) for u in range(len(heads)) for c in range(4) for j in range(NBLK)]
        scores, probs, sums = {}, {}, {}
        terms = [(n, t, d) for n in range(len(steps)) for t in range(4) for d in range(DH)]
        partial, state = {}, dict(terms=0, pairs=0)

        def emit(n, row, t, s0, s1):
            u, c, j = steps[n]
            p0, p1 = jnp.exp2(s0), jnp.exp2(s1)
            sums[u, c, t] = p0 + p1 if (u, c, t) not in sums else (sums[u, c, t] + p0) + p1
            probs[n, row, t] = _pack_pair(p0, p1)

        def vector_term():
            n, t, d = terms[state["terms"]]
            u, c, j = steps[n]
            _, keys, queries = heads[u][1]
            col = (4 * c + t) * 128
            q = jnp.broadcast_to(queries[d:d + 1, col:col + 128], (8, 128))
            for odd in range(2):
                term = keys[j, d, 8 * odd:8 * odd + 8, :] * q
                partial[odd] = term if d == 0 else partial[odd] + term
            if d == DH - 1:
                emit(n, 0, t, partial[0], partial[1])
            state["terms"] += 1

        def exponentials(n):
            u, c, j = steps[n]
            h, _, h_next, nxt = heads[u]
            s = scores.pop(n)
            for r in range(7):
                for t in range(4):
                    while state["terms"] < len(terms) and (state["terms"] + 6) * 28 <= state["pairs"] * 4 * DH:
                        vector_term()
                    emit(n, r + 1, t, _tile(s[16 * r:16 * r + 8], t), _tile(s[16 * r + 8:16 * r + 16], t))
                    state["pairs"] += 1
            while state["terms"] < len(terms) and terms[state["terms"]][0] <= n:
                vector_term()
            if j == NBLK - 1:
                for t in range(4):
                    lb[4 * c + t, pl.ds(pl.multiple_of(8 * h, 8), 8), :] = sums.pop((u, c, t))
            blocks = range(4 * c, 4 * c + 4)
            if j == 0:
                for block in blocks:
                    stage_keys(h_next, block, nxt[0])
            splat_keys(j, blocks, nxt[1])
            if j == 3:
                stage_queries(h_next, c, nxt[2])

        def weighted_values(n):
            u, c, j = steps[n]
            h = heads[u][0]
            p = jnp.concatenate([_lanes([probs.pop((n, r, t)) for t in range(4)]) for r in range(8)], axis=0)
            o = jnp.dot(_as_bf16(vw[j, h]), _as_bf16(p), preferred_element_type=f32)
            for t in range(4):
                ob[4 * c + t, h] = _tile(o, t) if j == 0 else ob[4 * c + t, h] + _tile(o, t)

        for n in range(len(steps) + 2):
            if n < len(steps):
                u, c, j = steps[n]
                h, (keys, _, _) = heads[u][:2]
                scores[n] = jnp.dot(_as_bf16(keys[j, 8:64, :]), q_operand(h, c), preferred_element_type=f32)
            if 0 <= n - 1 < len(steps):
                exponentials(n - 1)
            if n - 2 >= 0:
                weighted_values(n - 2)

    def fast_trip(i, carry):
        stages = ((krot, kb, qcur), (krot2, kb2, qcur2))
        first = HEADS_PER_TRIP * i
        fast_heads([(first + u, stages[u % 2], jnp.minimum(first + u + 1, H - 1), stages[1 - u % 2])
                    for u in range(HEADS_PER_TRIP)])
        return carry

    def guarded_head(h, carry):
        g, shift = h // 8, head_shift(h)

        def rotate(j, carry):
            krot[j] = pltpu.roll(kw[g, j], shift, axis=1)
            return carry

        jax.lax.fori_loop(0, NBLK, rotate, 0)

        def chunk(c, carry):
            q = q_operand(h, c)

            def block_scores(j):
                return jnp.dot(_as_bf16(krot[j]), q, preferred_element_type=f32)

            def running_max(j, m):
                return jnp.maximum(m, jnp.max(block_scores(j), axis=0, keepdims=True))

            m = jax.lax.fori_loop(0, NBLK, running_max, jnp.full((1, 512), -jnp.inf, f32))

            def accumulate(j, state):
                acc, total = state
                p = jnp.exp2(block_scores(j) - m)
                words = [_pack_pair(p[16 * r:16 * r + 8], p[16 * r + 8:16 * r + 16]) for r in range(8)]
                o = jnp.dot(_as_bf16(vw[j, h]), _as_bf16(jnp.concatenate(words, axis=0)),
                            preferred_element_type=f32)
                return acc + o, total + jnp.sum(p.reshape(16, 8, 512), axis=0)

            acc, total = jax.lax.fori_loop(
                0, NBLK, accumulate, (jnp.zeros((DH, 512), f32), jnp.zeros((8, 512), f32)))
            for t in range(4):
                ob[4 * c + t, h] = _tile(acc, t)
                lb[4 * c + t, pl.ds(pl.multiple_of(8 * h, 8), 8), :] = _tile(total, t)
            return carry

        return jax.lax.fori_loop(0, 4, chunk, carry)

    def full_attention():
        for j in range(NBLK):
            stage_keys(0, j, krot)
        for d in range(DH):
            splat_keys(d, range(NBLK), kb)
        for c in range(4):
            stage_queries(0, c, qcur)
        bound2 = jnp.max(norm2[0], axis=-1, keepdims=True) * jnp.max(norm2[1], axis=-1, keepdims=True)
        unsafe = jnp.max(jnp.where(bound2 <= SAFE_LOG2 * SAFE_LOG2, 0.0, 1.0))

        @pl.when(unsafe == 0.0)
        def _():
            jax.lax.fori_loop(0, H // HEADS_PER_TRIP, fast_trip, 0)

        @pl.when(unsafe != 0.0)
        def _():
            jax.lax.fori_loop(0, H, guarded_head, 0)

    def normalize_tasks(c):
        def task(y, t):
            b = 4 * c + t
            inv[c][t] = 1.0 / head_sums(lb.at[b], H)
            for h in range(H):
                scale = jnp.broadcast_to(inv[c][t, h:h + 1, :], (8, 128))
                even, odd = (ob[b, h, pl.ds(k, 8, stride=2), :] for k in range(2))
                words = _pack_pair(even * scale, odd * scale)
                oa[c][t, 8 * h:8 * h + 8, :] = words
            return words
        return [lambda y, t=t: task(y, t) for t in range(4)]

    def full_out(zero):
        for task in normalize_tasks(0):
            task(None)
        run(out_products(B_OUT, 0), normalize_tasks(1))
        run(out_products(B_OUT, 1), norm_tasks(0, zero) + normalize_tasks(2))
        run(out_products(B_OUT, 2), norm_tasks(1, zero) + normalize_tasks(3))
        run(out_products(B_OUT, 3), norm_tasks(2, zero))
        for task in norm_tasks(3, zero):
            task(None)

    def write_output():
        for c in (0, 2, 1, 3):
            for task in normalize_tasks(c):
                task(None)
        copies = []
        for j in range(4):
            for c in range(2):
                even, odd = project(B_OUT, oa, c, j * 128, 128), project(B_OUT, oa, c + 2, j * 128, 128)
                rows = pl.ds(j * 128, 128)
                for t in range(4):
                    words = _pack_pair(x_t[c][t, rows, :] + _tile(even, t), x_t[2 + c][t, rows, :] + _tile(odd, t))
                    io_words[j, pl.ds(4 * c + t, 128, stride=8), :] = words.T
            cp = pltpu.make_async_copy(io_buf.at[j], out_hbm.at[:, pl.ds(j * 128, 128)], out_sem.at[j])
            cp.start()
            copies.append(cp)
        for cp in copies:
            cp.wait()

    def dense_part(zero, first):
        def products(fn, c):
            size = 128 if fn is local_qkv else 256
            return [lambda part=part, row=row: fn(c, part, row, size) for part in range(3) for row in range(0, D, size)]

        def attention_task(par, i, g):
            return gated(qa[par], zero, lambda y: local_attention(par, i, g))

        def with_norm(c):
            outs = out_products(A_OUT, c)

            def last(product=outs[-1]):
                y = product()
                for task in norm_tasks(c, zero):
                    task(None)
                return y
            return outs[:-1] + [last]

        tasks = [[attention_task(par, i, g) for i in range(8) for g in range(4)] for par in range(2)]
        run(products(local_qkv, 0) + products(local_qkv, 1))
        if first:
            transpose_late_weights()
        l3, f0, f1, f2 = products(local_qkv, 3), *(products(full_qkv, c) for c in range(3))
        queue = products(local_qkv, 2) + l3[:6] + with_norm(0) + l3[6:]
        run(queue[:-1], tasks[0])
        run(queue[-1:])
        queue = f0[:4] + with_norm(1) + f0[4:] + f1[:5] + with_norm(2) + f1[5:]
        run(queue[:-1], tasks[1])
        run(queue[-1:] + f2[:5] + with_norm(3) + f2[5:] + products(full_qkv, 3))

    zero = (jnp.max(jnp.abs(x_t[0][0, 0:8, :])) < 0.0).astype(jnp.int32)
    dense_part(zero, True)
    full_attention()
    full_out(zero)
    dense_part(zero, False)
    full_attention()
    write_output()


@jax.jit
def pallas_interleave_layers__sliding_local_dilated__softmax_full_mha__prompt_kernel(
    A_x: jax.Array,
    A_wqkv: jax.Array,
    A_wo: jax.Array,
    B_x: jax.Array,
    B_wqkv: jax.Array,
    B_wo: jax.Array,
):
    del B_x
    vmem = pltpu.VMEM
    scratch = [
        vmem((4, S, 128), bf16),
        vmem((3, D, D), bf16),
        vmem((D, 3 * D), bf16),
        vmem((4, D, 128), bf16),
        vmem((D, D), bf16),
        vmem((4, H * PITCH, 128), f32),
        vmem((8, D // 2, D), u32),
        [vmem((5, D, 128), f32)] * 4,
        [vmem((4, D // 2, 128), u32)] * 4,
        [vmem((9, D, 128), f32)] * 2,
        [vmem((15, D, 128), f32)] * 2,
        [vmem((15, D, 128), f32)] * 2,
        [vmem((4, D // 2, 128), u32)] * 4,
        vmem((NBLK, H, DH, 128), f32),
        vmem((NBLK, H, 8, 128), u32),
        vmem((NBLK, H, 8, 128), u32),
        vmem((4, NBLK, 64, 128), u32),
        vmem((4, NBLK, 16, 128), f32),
        vmem((NBLK, 16, 128), f32),
        [vmem((4, 128, 128), f32)] * 4,
        [vmem((8 * H, 128), f32)] * 4,
        [vmem((4, H, 128), f32)] * 4,
        vmem((2, H, 128), f32),
        vmem((NBLK, H, DH, 128), f32),
        vmem((NBLK, 8 * H, 128), f32),
        vmem((NBLK, 64, 128), u32),
        vmem((NBLK, DH, 16, 128), f32),
        vmem((DH, S), f32),
        vmem((NBLK, 64, 128), u32),
        vmem((NBLK, DH, 16, 128), f32),
        vmem((DH, S), f32),
        pltpu.SemaphoreType.DMA((13,)),
        pltpu.SemaphoreType.DMA((4,)),
    ]
    out = pl.pallas_call(
        _kernel,
        out_shape=jax.ShapeDtypeStruct((S, D), bf16),
        in_specs=[pl.BlockSpec(memory_space=pl.ANY)] * 5,
        out_specs=pl.BlockSpec(memory_space=pl.ANY),
        scratch_shapes=scratch,
        compiler_params=pltpu.CompilerParams(
            vmem_limit_bytes=100 * 1024 * 1024,
            flags={"XLA_TPU_EVENLY_DISTRIBUTE_CRITICAL_NODES": True},
        ),
    )(A_x.reshape(S, D), A_wqkv, A_wo, B_wqkv, B_wo)
    return out.reshape(A_x.shape)
```
